```python
import os as _os
_os.environ.setdefault("JAX_PLATFORMS", "cpu")
import jax
import jax.numpy as jnp

def _softmax(x, axis=-1):
    return jax.nn.softmax(x, axis=axis)
def _gelu(x):
    return jax.nn.gelu(x, approximate=True)
def _silu(x):
    return jax.nn.silu(x)
def _sigmoid(x):
    return jax.nn.sigmoid(x)
def _layernorm(x, axis=-1, eps=1e-5):
    m = jnp.mean(x, axis=axis, keepdims=True)
    v = jnp.var(x, axis=axis, keepdims=True)
    return (x - m) / jnp.sqrt(v + eps)
def _scatter_add(tgt, idx, src, axis=0):
    return tgt.at[idx].add(src)
def _segment_sum(src, seg, n):
    return jax.ops.segment_sum(src, seg, n)
class _Rng:
    def __init__(self, key):
        self._k = key
    def _next(self):
        self._k, sub = jax.random.split(self._k)
        return sub
    def normal(self, shape):
        return jax.random.normal(self._next(), shape, dtype=jnp.bfloat16)
    def randint(self, lo, hi, shape):
        return jax.random.randint(self._next(), shape, lo, hi, dtype=jnp.int32)
    def uniform(self, shape, lo=0.0, hi=1.0):
        return jax.random.uniform(self._next(), shape, jnp.bfloat16, lo, hi)
    def permutation(self, n):
        return jax.random.permutation(self._next(), n)


kernel_name = 'standalone__seq2seq_rnn_t_joint__speech'

def setup_inputs():
    _rng = _Rng(jax.random.key(int.from_bytes(__import__("os").urandom(4), "little")))
    _w = (lambda a: (lambda t: t.astype(jnp.bfloat16) if jnp.issubdtype(t.dtype, jnp.floating) else t)(jnp.asarray(a)))
    B, T, D, K = 2, 1000, 512, 31
    U = 8
    sc = (1.0 / (K * D)) ** 0.5
    sd = (1.0 / D) ** 0.5
    return {
        "x": _w((lambda *s: _rng.normal(s) * 0.4)(B, T, D) * 0.5),
        "w1": _w((lambda *s: _rng.normal(s) * 1.6)(K, D, D) * sc),
        "w2": _w((lambda *s: _rng.normal(s) * 1.6)(K, D, D) * sc),
        "g": _w((lambda *s: _rng.normal(s) * 1.6)(B, U, D) * 0.5),
        "w_f": _w((lambda *s: _rng.normal(s) * 1.6)(D, D) * sd),
        "w_g": _w((lambda *s: _rng.normal(s) * 1.6)(D, D) * sd),
        "w_o": _w((lambda *s: _rng.normal(s) * 1.6)(D, D) * sd),
    }

def reference(x, w1, w2, g, w_f, w_g, w_o):
    B, T, D = x.shape
    K = w1.shape[0]
    pad = K // 2
    xp = jnp.pad(x, ((0,0),(pad,pad),(0,0)))
    h = jnp.zeros_like(x)
    for i in range(K):
        h = h + jnp.einsum("btc,cd->btd", xp[:, i:i+T, :], w1[i])
    h = _gelu(h)[:, ::2, :]
    T1 = h.shape[1]
    hp = jnp.pad(h, ((0,0),(pad,pad),(0,0)))
    f = jnp.zeros_like(h)
    for i in range(K):
        f = f + jnp.einsum("btc,cd->btd", hp[:, i:i+T1, :], w2[i])
    f = _gelu(f)[:, ::2, :]
    fe = jnp.einsum("btd,de->bte", f, w_f)
    ge = jnp.einsum("bud,de->bue", g, w_g)
    j = jnp.tanh(fe[:, :, None, :] + ge[:, None, :, :])
    return jnp.einsum("btud,dv->btuv", j, w_o)
```

```python
import itertools

import numpy as np
import jax
import jax.numpy as jnp
from jax import lax
import jax.experimental.pallas as pl
import jax.experimental.pallas.tpu as pltpu

f32, bf16 = jnp.float32, jnp.bfloat16
BT = np.array([[1, -1, 0], [0, 1, 0], [0, -1, 1]])
GM = np.array([[1, 0], [1, 1], [0, 1]])
AT = np.array([[1, 1, 0], [0, 1, 1]])

L1, L2 = 3, 2
P1, P2 = 2**L1, 2**L2
NK1, NK2 = 16 // P1, 16 // P2
T1, T2 = 500, 250
M1 = 64
M2 = 64
R1 = P1 * (M1 + 8) + 2 * P1 + 8
R2 = 16 + M1 + 32
JT = 50
NCH = T2 // JT
G1 = ((0, 2), (2, 4), (4, 8), (8, 16))


def _gelu(x):
    c = np.float32(np.sqrt(2 / np.pi))
    return 0.5 * x * (1.0 + jnp.tanh(c * (x + np.float32(0.044715) * x * x * x)))


def _lin(idx):
    r = 0
    for i in idx:
        r = 2 * r + i
    return r


def _xform(cur, mat, L):
    for ax in range(L):
        new = {}
        for o in sorted({k[:ax] + k[ax + 1:] for k in cur}):
            for r in range(mat.shape[0]):
                vs = [(mat[r, i], cur[o[:ax] + (i,) + o[ax:]])
                      for i in range(mat.shape[1]) if mat[r, i]]
                vs.sort(key=lambda t: -t[0])
                val = vs[0][1]
                for c, v in vs[1:]:
                    val = val + v if c > 0 else val - v
                new[o[:ax] + (r,) + o[ax:]] = val
        cur = new
    return cur


def _streams(L):
    def terms(s):
        return sorted(_lin(q) for q in itertools.product(range(2), repeat=L)
                      if all(GM[a, b] for a, b in zip(s, q)))
    S = list(itertools.product(range(3), repeat=L))
    S.sort(key=lambda s: (max(terms(s)), len(terms(s)), terms(s)))
    return S, [terms(s) for s in S]


S1, TAPS1 = _streams(L1)
S2, TAPS2 = _streams(L2)


def _kernel(x_h, w1_h, w2_h, g_h, wf_h, wg_h, wo_h, o_h,
            xv, Wa, Wb, gv, wfv, wgv, wov, Xs, Hs, Ds, acc, FE, GE, ob,
            sx, s1, s2, sm, so):
    mo = pl.multiple_of

    def wcopy(src, dst, sem, a, b):
        lo, hi = max(2 * a - 1, 0), 2 * b - 1
        return pltpu.make_async_copy(src.at[pl.ds(lo, hi - lo)],
                                     dst.at[pl.ds(lo + 1, hi - lo)], sem)

    cx = [pltpu.make_async_copy(x_h.at[b], xv.at[b], sx.at[b]) for b in range(2)]
    c1 = [wcopy(w1_h, Wa, s1.at[i], a, b) for i, (a, b) in enumerate(G1)]
    c2 = [wcopy(w2_h, Wb, s2.at[i], 8 * i, 8 * i + 8) for i in range(2)]
    cm = [pltpu.make_async_copy(a, b, sm.at[i]) for i, (a, b) in
          enumerate([(g_h, gv), (wf_h, wfv), (wg_h, wgv), (wo_h, wov)])]
    for c in cx + c1[:1]:
        c.start()
    Wa[0] = jnp.zeros((512, 512), bf16)
    Wb[0] = jnp.zeros((512, 512), bf16)
    for b in range(2):
        for c in range(4):
            for hh in range(2):
                Xs[hh, b, c, 0:8, :] = jnp.zeros((8, 128), f32)
                Xs[hh, b, c, 504:R1, :] = jnp.zeros((R1 - 504, 128), f32)
            for p in range(P1):
                Hs[p, b, c, 8:16, :] = jnp.zeros((8, 128), f32)
                Hs[p, b, c, 16 + M1:R2, :] = jnp.zeros((R2 - 16 - M1, 128), f32)

    def prep(load, L, S, M, b, hh, c):
        for v0 in range(0, M + 8, 8):
            zr = {r: load(hh, b, c, r, v0) for r in range(2**(L + 1) - 1)}
            ds = _xform({i: zr[_lin(i)] for i in itertools.product(range(3), repeat=L)}, BT, L)
            for i, s in enumerate(S):
                Ds[i, hh * 4 + c, pl.ds(2 * v0 + b, 8, stride=2), :] = ds[s]

    def load1(hh, b, c, r, v0):
        return Xs[hh, b, c, pl.ds(P1 * v0 + r, 8, stride=P1), :]

    def load2(hh, b, c, r, v0):
        s0 = 2 * (P2 * v0 + r - 8)
        return Hs[s0 % P1 + hh, b, c, pl.ds(16 + s0 // P1, 8, stride=2 * P2 // P1), :]

    def xbody(i, _):
        b, c = i >> 2, i & 3
        pl.when(i == 0)(cx[0].wait)
        pl.when(i == 4)(cx[1].wait)

        @pl.when(i == 7)
        def _():
            c1[1].start()
            c1[2].start()
        u = pltpu.bitcast(xv[b, :, pl.ds(mo(c * 128, 128), 128)], jnp.uint32)
        Xs[0, b, c, 8:508, :] = pltpu.bitcast(u << 16, f32)
        Xs[1, b, c, 8:508, :] = pltpu.bitcast(u & jnp.uint32(0xFFFF0000), f32)
        prep(load1, L1, S1, M1, b, 0, c)
        prep(load1, L1, S1, M1, b, 1, c)
    lax.fori_loop(0, 8, xbody, None)

    def mm(W, P, M, i, k, taps):
        r = None
        for t in range(8):
            hh, r0 = t // 4, (t % 4) * 128
            lhs = jnp.concatenate([Ds[i, t, pl.ds(2 * k + b, M, stride=2), :]
                                   for b in range(2)], axis=0).astype(bf16)
            ws = [W[2 * (P * k + q) + hh, r0:r0 + 128, :] for q in taps]
            if len(ws) == 1:
                w = ws[0]
            else:
                ws = [a.astype(f32) for a in ws]
                while len(ws) > 1:
                    ws = [ws[a] + ws[a + 1] for a in range(0, len(ws), 2)]
                w = ws[0].astype(bf16)
            d = jnp.dot(lhs, w, preferred_element_type=f32)
            r = d if r is None else r + d
        acc[i] = jnp.where(k == 0, 0.0, acc[i]) + r

    starts = {(0, 9): c1[3:], (0, 22): c2[:1], (1, 6): c2[1:], (1, 18): cm}

    def start_all(cs):
        for c in cs:
            c.start()

    def conv1(k, _):
        seen = 0
        for i in range(len(S1)):
            while seen < 3 and G1[seen][0] <= max(TAPS1[i]):
                pl.when(k == 0)(c1[seen].wait)
                seen += 1
            if i == 0:
                pl.when(k == 1)(c1[3].wait)
            for kk in range(NK1):
                if (kk, i) in starts:
                    pl.when(k == kk)(lambda cs=starts[kk, i]: start_all(cs))
            mm(Wa, P1, M1, i, k, TAPS1[i])
    lax.fori_loop(0, NK1, conv1, None)

    def hbody(u, _):
        b, c = u >> 2, u & 3
        ms = {s: acc[i, pl.ds(mo(b * M1, 16), M1), pl.ds(mo(c * 128, 128), 128)]
              for i, s in enumerate(S1)}
        row = lax.broadcasted_iota(jnp.int32, (M1, 128), 0)
        for p_idx, y in _xform(ms, AT, L1).items():
            p = _lin(p_idx)
            Hs[p, b, c, 16:16 + M1, :] = jnp.where(row < (T1 - p + P1 - 1) // P1, _gelu(y), 0.0)
        prep(load2, L2, S2, M2, b, 0, c)
        prep(load2, L2, S2, M2, b, 1, c)
    lax.fori_loop(0, 8, hbody, None)

    for c in c2:
        c.wait()

    def conv2(k, _):
        for i in range(len(S2)):
            mm(Wb, P2, M2, i, k, TAPS2[i])
    lax.fori_loop(0, NK2, conv2, None)

    for c in cm:
        c.wait()
    for b in range(2):
        GE[b] = jnp.dot(gv[b], wgv[...], preferred_element_type=f32)

    def febody(b, _):
        ms = {s: acc[i, pl.ds(mo(b * M2, 16), M2), :] for i, s in enumerate(S2)}
        ys = _xform(ms, AT, L2)
        f = jnp.concatenate([_gelu(ys[p]).astype(bf16)
                             for p in itertools.product(range(2), repeat=L2)], axis=0)
        fe = jnp.dot(f, wfv[...], preferred_element_type=f32)
        for p in range(P2):
            for c in range(4):
                FE[b, c, pl.ds(p, M2, stride=P2), :] = fe[p * M2:(p + 1) * M2, c * 128:(c + 1) * 128]
    lax.fori_loop(0, 2, febody, None)

    def jbody(i, _):
        b = lax.div(i, jnp.int32(NCH))
        t0 = (i - b * NCH) * JT
        fe = jnp.concatenate([FE[b, c, pl.ds(t0, JT), :] for c in range(4)], axis=1)
        j = jnp.tanh(fe[:, None, :] + GE[b][None, :, :]).reshape(JT * 8, 512)
        o = jnp.dot(j.astype(bf16), wov[...], preferred_element_type=f32)
        ob[i] = o.reshape(JT, 8, 512).astype(bf16)
        pltpu.make_async_copy(ob.at[i], o_h.at[b, pl.ds(t0, JT)], so.at[0]).start()
    lax.fori_loop(0, 2 * NCH, jbody, None)
    for i in range(2 * NCH):
        pltpu.make_async_copy(ob.at[i], o_h.at[i // NCH, pl.ds((i % NCH) * JT, JT)], so.at[0]).wait()


@jax.jit
def pallas_standalone__seq2seq_rnn_t_joint__speech_kernel(
    x: jax.Array,
    w1: jax.Array,
    w2: jax.Array,
    g: jax.Array,
    w_f: jax.Array,
    w_g: jax.Array,
    w_o: jax.Array,
):
    V, DMA = pltpu.VMEM, pltpu.SemaphoreType.DMA
    scratch = [
        V((2, 1000, 512), bf16), V((32, 512, 512), bf16), V((32, 512, 512), bf16),
        V((2, 8, 512), bf16), V((512, 512), bf16), V((512, 512), bf16), V((512, 512), bf16),
        V((2, 2, 4, R1, 128), f32), V((P1, 2, 4, R2, 128), f32),
        V((len(S1), 8, 2 * (M1 + 8), 128), f32), V((len(S1), 2 * M1, 512), f32),
        V((2, 4, P2 * M2, 128), f32), V((2, 8, 512), f32), V((2 * NCH, JT, 8, 512), bf16),
        DMA((2,)), DMA((len(G1),)), DMA((2,)), DMA((4,)), DMA((1,)),
    ]
    return pl.pallas_call(
        _kernel,
        out_shape=jax.ShapeDtypeStruct((2, T2, 8, 512), bf16),
        in_specs=[pl.BlockSpec(memory_space=pl.ANY)] * 7,
        out_specs=pl.BlockSpec(memory_space=pl.ANY),
        scratch_shapes=scratch,
        compiler_params=pltpu.CompilerParams(vmem_limit_bytes=110 * 1024 * 1024),
    )(x, w1, w2, g, w_f, w_g, w_o)
```
